```python
import os as _os
_os.environ.setdefault("JAX_PLATFORMS", "cpu")
import jax
import jax.numpy as jnp

def _softmax(x, axis=-1):
    return jax.nn.softmax(x, axis=axis)
def _gelu(x):
    return jax.nn.gelu(x, approximate=True)
def _silu(x):
    return jax.nn.silu(x)
def _sigmoid(x):
    return jax.nn.sigmoid(x)
def _layernorm(x, axis=-1, eps=1e-5):
    m = jnp.mean(x, axis=axis, keepdims=True)
    v = jnp.var(x, axis=axis, keepdims=True)
    return (x - m) / jnp.sqrt(v + eps)
def _scatter_add(tgt, idx, src, axis=0):
    return tgt.at[idx].add(src)
def _segment_sum(src, seg, n):
    return jax.ops.segment_sum(src, seg, n)
class _Rng:
    def __init__(self, key):
        self._k = key
    def _next(self):
        self._k, sub = jax.random.split(self._k)
        return sub
    def normal(self, shape):
        return jax.random.normal(self._next(), shape, dtype=jnp.bfloat16)
    def randint(self, lo, hi, shape):
        return jax.random.randint(self._next(), shape, lo, hi, dtype=jnp.int32)
    def uniform(self, shape, lo=0.0, hi=1.0):
        return jax.random.uniform(self._next(), shape, jnp.bfloat16, lo, hi)
    def permutation(self, n):
        return jax.random.permutation(self._next(), n)


kernel_name = 'gated_mix__linear_attn_block__mixer_token_mlp__prompt'

def setup_inputs():
    _rng = _Rng(jax.random.key(int.from_bytes(__import__("os").urandom(4), "little")))
    _w = (lambda a: (lambda t: t.astype(jnp.bfloat16) if jnp.issubdtype(t.dtype, jnp.floating) else t)(jnp.asarray(a)))
    def _A_setup():
        B, S, D = 1, 2048, 512
        return {
            "x": _w((lambda *s: _rng.normal(s) * 0.05)(B, S, D)),
            "wqkv": _w((lambda *s: _rng.normal(s) * 0.8)(D, 3 * D)),
            "wo": _w((lambda *s: _rng.normal(s) * 0.05)(D, D)),
        }
    _A_in = _A_setup()

    def _B_setup():
        B, S, D, F = 1, 2048, 512, 1792
        return {
            "x": _w((lambda *s: _rng.normal(s) * 0.05)(B, S, D)),
            "w1": _w((lambda *s: _rng.normal(s) * 0.1)(S, F) * (S ** -0.5)),
            "b1": _w((lambda *s: _rng.normal(s) * 0.1)(F) * 0.02),
            "w2": _w((lambda *s: _rng.normal(s) * 0.1)(F, S) * (F ** -0.5)),
            "b2": _w((lambda *s: _rng.normal(s) * 0.1)(S) * 0.02),
        }
    _B_in = _B_setup()

    return {
        "A_x": _A_in["x"],
        "A_wqkv": _A_in["wqkv"],
        "A_wo": _A_in["wo"],
        "B_x": _B_in["x"],
        "B_w1": _B_in["w1"],
        "B_b1": _B_in["b1"],
        "B_w2": _B_in["w2"],
        "B_b2": _B_in["b2"],
        "gate_w": _w((lambda *s: _rng.normal(s) * 0.05)(512) * 16.0),
    }

def reference(A_x, A_wqkv, A_wo, B_x, B_w1, B_b1, B_w2, B_b2, gate_w):
    def _A_ref(x, wqkv, wo):
        B, S, D = x.shape
        H = 32; Dh = D // H
        qkv = (lambda x, *d: x.transpose(*d))((x @ wqkv).reshape(B, S, 3, H, Dh), 2, 0, 3, 1, 4)
        q, k, v = qkv[0], qkv[1], qkv[2]
        phi = lambda t: jnp.where(t > 0, t + 1, jnp.exp(t)) + 1e-6
        pq, pk = phi(q), phi(k)
        kv = jnp.einsum("bhsd,bhse->bhde", pk, v)
        z = jnp.einsum("bhsd->bhd", pk)
        num = jnp.einsum("bhqd,bhde->bhqe", pq, kv)
        den = jnp.einsum("bhqd,bhd->bhq", pq, z)[..., None] + 1e-6
        o = num / den
        return (lambda x, *d: x.transpose(*d))(o, 0, 2, 1, 3).reshape(B, S, D) @ wo

    def _B_ref(x, w1, b1, w2, b2):
        B, S, D = x.shape
        h = _layernorm(x, axis=-1)
        u = jnp.einsum("bsd,sf->bdf", h, w1) + b1
        u = _gelu(u)
        y = jnp.einsum("bdf,fs->bds", u, w2) + b2
        return (lambda x, *d: x.transpose(*d))(y, 0, 2, 1)

    x = A_x
    g = _sigmoid((x * gate_w).sum(-1, keepdims=True))
    a = _A_ref(x, A_wqkv, A_wo)
    b = _B_ref(x, B_w1, B_b1, B_w2, B_b2)
    return g * a + (1 - g) * b
```

```python
import jax
import jax.numpy as jnp
import jax.experimental.pallas as pl
import jax.experimental.pallas.tpu as pltpu

_HEAD_DIM = 16
_GROUP = 128


def _phi(t):
    return jnp.where(t > 0, t + 1.0, jnp.exp(t)) + 1e-6


def _gelu_tanh(x):
    c = 0.7978845608028654
    return 0.5 * x * (1.0 + jnp.tanh(c * (x + 0.044715 * (x * x * x))))


def _make_kernel(s, d, f, ts):
    n = s // ts
    n_groups = d // _GROUP
    f32 = jnp.float32
    bf16 = jnp.bfloat16

    SEM_X = 0
    SEM_W1 = n
    SEM_W2 = 2 * n
    SEM_OUT = 3 * n
    SEM_WQKV = 4 * n
    SEM_WO = 4 * n + 3
    n_sems = 4 * n + 4

    def kernel(x_hbm, wqkv_hbm, wo_hbm, w1_hbm, b1_ref, w2_hbm, b2_ref, gw_ref,
               o_hbm,
               x_buf, wqkv_buf, wo_buf, w1_buf, w2_buf, o_buf,
               pq_scr, u_scr, ua_scr, m_scr, sems):

        def cp_x(t):
            return pltpu.make_async_copy(
                x_hbm.at[pl.ds(t * ts, ts), :], x_buf.at[pl.ds(t * ts, ts), :],
                sems.at[SEM_X + t])

        def cp_w1(t):
            return pltpu.make_async_copy(
                w1_hbm.at[pl.ds(t * ts, ts), :], w1_buf.at[pl.ds(t * ts, ts), :],
                sems.at[SEM_W1 + t])

        def cp_w2(t):
            return pltpu.make_async_copy(
                w2_hbm.at[:, pl.ds(t * ts, ts)], w2_buf.at[:, pl.ds(t * ts, ts)],
                sems.at[SEM_W2 + t])

        def cp_out(t):
            return pltpu.make_async_copy(
                o_buf.at[pl.ds(t * ts, ts), :], o_hbm.at[pl.ds(t * ts, ts), :],
                sems.at[SEM_OUT + t])

        def cp_wqkv(j):
            return pltpu.make_async_copy(
                wqkv_hbm.at[:, pl.ds(j * d, d)], wqkv_buf.at[:, pl.ds(j * d, d)],
                sems.at[SEM_WQKV + j])
        cp_wo = pltpu.make_async_copy(wo_hbm, wo_buf, sems.at[SEM_WO])

        def group_mask():
            r = jax.lax.broadcasted_iota(jnp.int32, (_GROUP, _GROUP), 0) // _HEAD_DIM
            c = jax.lax.broadcasted_iota(jnp.int32, (_GROUP, _GROUP), 1) // _HEAD_DIM
            return r == c

        cp_x(0).start()
        for j in range(3):
            cp_wqkv(j).start()
        for t in range(1, n):
            cp_x(t).start()
            cp_w1(t - 1).start()
        cp_w1(n - 1).start()
        cp_wo.start()
        for t in range(n):
            cp_w2(t).start()

        fc = 256
        n_fc = f // fc
        b1v = b1_ref[...].reshape(1, f).astype(f32)

        def u_chunk(tp, hT, c, last):
            cols = slice(c * fc, (c + 1) * fc)
            prow = slice(tp * ts, (tp + 1) * ts)
            up = jnp.dot(hT, w1_buf[prow, cols], preferred_element_type=f32)
            if tp > 0:
                up = up + u_scr[:, cols]
            if last:
                ua_scr[:, cols] = _gelu_tanh(up + b1v[:, cols]).astype(bf16)
            else:
                u_scr[:, cols] = up

        kvs = [None] * n_groups
        z = None
        hT_prev = None
        for t in range(n):
            cp_x(t).wait()
            rows = slice(t * ts, (t + 1) * ts)
            xb = x_buf[rows, :]
            x = xb.astype(f32)

            if t == 0:
                cp_wqkv(0).wait()
            q = jnp.dot(xb, wqkv_buf[:, 0:d], preferred_element_type=f32)
            pq_scr[rows, :] = _phi(q).astype(bf16)
            if t == 0:
                cp_wqkv(1).wait()
            pk = _phi(jnp.dot(xb, wqkv_buf[:, d:2 * d], preferred_element_type=f32))
            pkb = pk.astype(bf16)
            if t == 0:
                cp_wqkv(2).wait()
            vb = jnp.dot(xb, wqkv_buf[:, 2 * d:3 * d],
                         preferred_element_type=f32).astype(bf16)
            zs = jnp.sum(pk, axis=0, keepdims=True)
            z = zs if z is None else z + zs

            mu = jnp.mean(x, axis=-1, keepdims=True)
            xc = x - mu
            var = jnp.mean(xc * xc, axis=-1, keepdims=True)
            h = (xc * jax.lax.rsqrt(var + 1e-5)).astype(bf16)
            hT = jnp.transpose(h)

            if t > 0:
                cp_w1(t - 1).wait()
            c = 0
            for g in range(n_groups):
                sl = slice(g * _GROUP, (g + 1) * _GROUP)
                kvg = jax.lax.dot_general(
                    pkb[:, sl], vb[:, sl], (((0,), (0,)), ((), ())),
                    preferred_element_type=f32)
                kvs[g] = kvg if kvs[g] is None else kvs[g] + kvg
                if t > 0:
                    c_end = ((g + 1) * n_fc) // n_groups
                    while c < c_end:
                        u_chunk(t - 1, hT_prev, c, False)
                        c += 1
            hT_prev = hT

        msk = group_mask()
        cp_wo.wait()
        for g in range(n_groups):
            sl = slice(g * _GROUP, (g + 1) * _GROUP)
            kvg = jnp.where(msk, kvs[g], 0.0).astype(bf16)
            m_scr[sl, :] = jnp.dot(kvg, wo_buf[sl, :],
                                   preferred_element_type=f32).astype(bf16)
        zms = []
        for g in range(n_groups):
            sl = slice(g * _GROUP, (g + 1) * _GROUP)
            zc = jnp.transpose(jnp.broadcast_to(z[:, sl], (_GROUP, _GROUP)))
            zms.append(jnp.where(msk, zc, 0.0).astype(bf16))
        cp_w1(n - 1).wait()
        for c in range(n_fc):
            u_chunk(n - 1, hT_prev, c, True)

        b2v = b2_ref[...].reshape(1, s).astype(f32)
        for t in range(n):
            rows = slice(t * ts, (t + 1) * ts)
            x = x_buf[rows, :].astype(f32)
            gl = jnp.sum(x * gw_ref[...].reshape(1, d).astype(f32), axis=-1, keepdims=True)
            gate = 1.0 / (1.0 + jnp.exp(-gl))

            pq = pq_scr[rows, :]
            parts = []
            bs = []
            nc = n_groups
            sc = ts // nc
            cp_w2(t).wait()
            for g in range(n_groups):
                sl = slice(g * _GROUP, (g + 1) * _GROUP)
                den = jnp.dot(pq[:, sl], zms[g], preferred_element_type=f32) + 1e-6
                parts.append((pq[:, sl].astype(f32) / den).astype(bf16))
                c0 = t * ts + g * sc
                yc = jnp.dot(ua_scr[...], w2_buf[:, c0:c0 + sc],
                             preferred_element_type=f32)
                yc = yc + b2v[:, c0:c0 + sc]
                bs.append(yc.T)
            pqn = jnp.concatenate(parts, axis=1)
            a = jnp.dot(pqn, m_scr[...], preferred_element_type=f32)
            b = jnp.concatenate(bs, axis=0)
            o_buf[rows, :] = (gate * a + (1.0 - gate) * b).astype(o_buf.dtype)
            cp_out(t).start()

        for t in range(n):
            cp_out(t).wait()

    return kernel, n_sems


@jax.jit
def pallas_gated_mix__linear_attn_block__mixer_token_mlp__prompt_kernel(
    A_x: jax.Array,
    A_wqkv: jax.Array,
    A_wo: jax.Array,
    B_x: jax.Array,
    B_w1: jax.Array,
    B_b1: jax.Array,
    B_w2: jax.Array,
    B_b2: jax.Array,
    gate_w: jax.Array,
):
    bsz, s, d = A_x.shape
    f = B_w1.shape[1]
    assert bsz == 1
    ts = 512

    x2 = A_x.reshape(s, d)
    b1 = B_b1
    b2 = B_b2
    gw = gate_w

    kernel, n_sems = _make_kernel(s, d, f, ts)
    any_spec = pl.BlockSpec(memory_space=pl.ANY)
    vmem_spec = pl.BlockSpec(memory_space=pltpu.VMEM)
    out = pl.pallas_call(
        kernel,
        in_specs=[any_spec, any_spec, any_spec, any_spec, vmem_spec, any_spec,
                  vmem_spec, vmem_spec],
        out_specs=any_spec,
        out_shape=jax.ShapeDtypeStruct((s, d), A_x.dtype),
        scratch_shapes=[
            pltpu.VMEM((s, d), jnp.bfloat16),
            pltpu.VMEM((d, 3 * d), jnp.bfloat16),
            pltpu.VMEM((d, d), jnp.bfloat16),
            pltpu.VMEM((s, f), jnp.bfloat16),
            pltpu.VMEM((f, s), jnp.bfloat16),
            pltpu.VMEM((s, d), jnp.bfloat16),
            pltpu.VMEM((s, d), jnp.bfloat16),
            pltpu.VMEM((d, f), jnp.float32),
            pltpu.VMEM((d, f), jnp.bfloat16),
            pltpu.VMEM((d, d), jnp.bfloat16),
            pltpu.SemaphoreType.DMA((n_sems,)),
        ],
        compiler_params=pltpu.CompilerParams(
            vmem_limit_bytes=100 * 1024 * 1024,
        ),
    )(x2, A_wqkv, A_wo, B_w1, b1, B_w2, b2, gw)
    return out.reshape(bsz, s, d)
```
